```python
import jax
import jax.numpy as jnp

def _softmax(x, axis=-1):
    return jax.nn.softmax(x, axis=axis)

def _gelu(x):
    return jax.nn.gelu(x, approximate=True)

def _silu(x):
    return jax.nn.silu(x)

def _sigmoid(x):
    return jax.nn.sigmoid(x)

def _layernorm(x, axis=-1, eps=1e-05):
    m = jnp.mean(x, axis=axis, keepdims=True)
    v = jnp.var(x, axis=axis, keepdims=True)
    return (x - m) / jnp.sqrt(v + eps)

def _scatter_add(tgt, idx, src, axis=0):
    return tgt.at[idx].add(src)

def _segment_sum(src, seg, n):
    return jax.ops.segment_sum(src, seg, n)

class _Rng:

    def __init__(self, key):
        self._k = key

    def _next(self):
        self._k, sub = jax.random.split(self._k)
        return sub

    def normal(self, shape):
        return jax.random.normal(self._next(), shape, dtype=jnp.bfloat16)

    def randint(self, lo, hi, shape):
        return jax.random.randint(self._next(), shape, lo, hi, dtype=jnp.int32)

    def uniform(self, shape, lo=0.0, hi=1.0):
        return jax.random.uniform(self._next(), shape, jnp.bfloat16, lo, hi)

    def permutation(self, n):
        return jax.random.permutation(self._next(), n)
kernel_name = 'adaLN_cond__mha_block_cached__moe_arch_mod__decode'

def setup_inputs():
    _rng = _Rng(jax.random.key(int.from_bytes(__import__("os").urandom(4), "little")))
    _w = lambda a: (lambda t: t.astype(jnp.bfloat16) if jnp.issubdtype(t.dtype, jnp.floating) else t)(jnp.asarray(a))

    def _A_setup():
        B, Sq, D = (4, 1, 448)
        H, Sk, Dh = (16, 16384, 256)
        return {'x': _w((lambda *s: _rng.normal(s) * 0.05)(B, Sq, D)), 'k_cache': _w((lambda *s: _rng.normal(s) * 0.05)(B, H, Sk, Dh)), 'v_cache': _w((lambda *s: _rng.normal(s) * 0.05)(B, H, Sk, Dh)), 'wq': _w((lambda *s: _rng.normal(s) * 0.05)(D, H * Dh) * D ** (-0.5)), 'wo': _w((lambda *s: _rng.normal(s) * 0.05)(H * Dh, D) * (H * Dh) ** (-0.5))}
    _A_in = _A_setup()

    def _B_setup():
        B, S, D, F, C = (4, 1, 448, 1792, 1)
        return {'x': _w((lambda *s: _rng.normal(s) * 0.05)(B, S, D)), 'w_r': _w((lambda *s: _rng.normal(s) * 0.05)(D)), 'w_gate': _w((lambda *s: _rng.normal(s) * 0.05)(D, F)), 'w_up': _w((lambda *s: _rng.normal(s) * 0.05)(D, F)), 'w_down': _w((lambda *s: _rng.normal(s) * 0.05)(F, D))}
    _B_in = _B_setup()
    return {'A_x': _A_in['x'], 'A_k_cache': _A_in['k_cache'], 'A_v_cache': _A_in['v_cache'], 'A_wq': _A_in['wq'], 'A_wo': _A_in['wo'], 'B_x': _B_in['x'], 'B_w_r': _B_in['w_r'], 'B_w_gate': _B_in['w_gate'], 'B_w_up': _B_in['w_up'], 'B_w_down': _B_in['w_down'], 'c': _w((lambda *s: _rng.normal(s) * 0.05)(4, 448)), 'w_mod': _w((lambda *s: _rng.normal(s) * 0.05)(448, 6 * 448) * 448 ** (-0.5))}

def reference(A_x, A_k_cache, A_v_cache, A_wq, A_wo, B_x, B_w_r, B_w_gate, B_w_up, B_w_down, c, w_mod):

    def _A_ref(x, k_cache, v_cache, wq, wo):
        B, Sq, D = x.shape
        H, Dh = (16, 256)
        q = (lambda x, *d: x.transpose(*d))((x @ wq).reshape(B, Sq, H, Dh), 0, 2, 1, 3)
        scores = jnp.einsum('bhqd,bhkd->bhqk', q, k_cache) * Dh ** (-0.5)
        p = _softmax(scores, axis=-1)
        o = jnp.einsum('bhqk,bhkd->bhqd', p, v_cache)
        return (lambda x, *d: x.transpose(*d))(o, 0, 2, 1, 3).reshape(B, Sq, H * Dh) @ wo

    def _B_ref(x, w_r, w_gate, w_up, w_down):
        B, S, D = x.shape
        C = 1
        r = x @ w_r
        idx = jnp.argsort(-r, axis=-1)[:, :C]
        idx_e = jnp.repeat(idx.reshape(B, C, 1), D, axis=2)
        x_sel = jnp.take_along_axis(x, idx_e, axis=1)
        g = _silu(x_sel @ w_gate)
        u = x_sel @ w_up
        y = g * u @ w_down
        r_sel = _sigmoid(jnp.take_along_axis(r, idx, axis=1))
        y = y * r_sel.reshape(B, C, 1)
        b_off = (jnp.arange(B) * S).reshape(B, 1)
        flat_idx = (idx + b_off).reshape(B * C)
        zero = (x * 0.0).reshape(B * S, D)
        upd = _scatter_add(zero, flat_idx, y.reshape(B * C, D), axis=0)
        return x + upd.reshape(B, S, D)
    x = A_x
    mod = (_silu(c) @ w_mod).reshape(c.shape[0], 6, 1, -1)
    sa, ca, ga, sb, cb, gb = (mod[:, 0].copy(), mod[:, 1].copy(), mod[:, 2].copy(), mod[:, 3].copy(), mod[:, 4].copy(), mod[:, 5].copy())
    h = _layernorm(x, axis=-1) * (1 + ca) + sa
    x = x + ga * _A_ref(h, A_k_cache, A_v_cache, A_wq, A_wo)
    h = _layernorm(x, axis=-1) * (1 + cb) + sb
    x = x + gb * _B_ref(h, B_w_r, B_w_gate, B_w_up, B_w_down)
    return x
```

```python
import functools

import jax
import jax.numpy as jnp
import jax.experimental.pallas as pl
import jax.experimental.pallas.tpu as pltpu

B, D, H, SK, DH, F = 4, 448, 16, 16384, 256, 1792
MP = 8


def _silu(v):
    return v * (1.0 / (1.0 + jnp.exp(-v)))


def _layernorm(v):
    m = jnp.mean(v, axis=-1, keepdims=True)
    d = v - m
    var = jnp.mean(d * d, axis=-1, keepdims=True)
    return d / jnp.sqrt(var + 1e-5)


def _pad_rows(v):
    return jnp.concatenate([v, jnp.zeros((MP - v.shape[0], v.shape[1]), v.dtype)], axis=0)


def _kernel(x_hbm, c_hbm, wr_hbm,
            k_hbm, v_hbm, wq_hbm, wo_hbm, wg_hbm, wu_hbm, wd_hbm, wm_hbm,
            out_hbm,
            x_ref, c_ref, wr_ref, out_ref,
            kbuf, vbuf, wq_v, wo_v, wg_v, wu_v, wd_v, wm_v, q_s, o_s,
            ksem, vsem, wsem, *, bs, nbuf):
    ns = SK // bs
    total = B * H * ns
    f32 = jnp.float32
    bf16 = jnp.bfloat16

    def kcopy(j, slot):
        return pltpu.make_async_copy(k_hbm.at[pl.ds(j * bs, bs), :], kbuf.at[slot], ksem.at[slot])

    def vcopy(j, slot):
        return pltpu.make_async_copy(v_hbm.at[pl.ds(j * bs, bs), :], vbuf.at[slot], vsem.at[slot])

    wm_c = pltpu.make_async_copy(wm_hbm, wm_v, wsem.at[0])
    wq_c = pltpu.make_async_copy(wq_hbm, wq_v, wsem.at[1])
    wo_c = pltpu.make_async_copy(wo_hbm, wo_v, wsem.at[2])
    wg_c = pltpu.make_async_copy(wg_hbm, wg_v, wsem.at[3])
    wu_c = pltpu.make_async_copy(wu_hbm, wu_v, wsem.at[4])
    wd_c = pltpu.make_async_copy(wd_hbm, wd_v, wsem.at[5])

    x_c = pltpu.make_async_copy(x_hbm, x_ref, wsem.at[6])
    c_c = pltpu.make_async_copy(c_hbm, c_ref, wsem.at[7])
    wr_c = pltpu.make_async_copy(wr_hbm, wr_ref, wsem.at[8])
    x_c.start()
    c_c.start()
    wr_c.start()
    wm_c.start()
    wq_c.start()
    for j in range(nbuf):
        kcopy(j, j).start()
        vcopy(j, j).start()
    wo_c.start()
    wg_c.start()
    wu_c.start()
    wd_c.start()

    x_c.wait()
    c_c.wait()
    x = _pad_rows(x_ref[...].astype(f32))
    c = _pad_rows(c_ref[...].astype(f32))
    sc = _silu(c).astype(bf16)
    wm_c.wait()
    mod = jnp.dot(sc, wm_v[...], preferred_element_type=f32)
    sa, ca, ga, sb, cb, gb = [mod[:, i * D:(i + 1) * D] for i in range(6)]
    h = _layernorm(x) * (1.0 + ca) + sa
    wq_c.wait()
    q = jnp.dot(h.astype(bf16), wq_v[...], preferred_element_type=f32)
    q = q.astype(bf16)
    for hh in range(H):
        q_s[hh] = q[:, hh * DH:(hh + 1) * DH]

    scale = DH ** -0.5
    row = jax.lax.broadcasted_iota(jnp.int32, (MP, DH), 0)

    def head_loop(hh, _):
        o_s[hh] = jnp.zeros((MP, DH), f32)
        qh = q_s[hh]

        def batch_loop(b, _):
            base = (b * H + hh) * ns

            def chunk(i, carry):
                m, l, acc = carry
                step = (hh * B + b) * ns + i
                slot = jax.lax.rem(step, nbuf)
                kcopy(0, slot).wait()
                s = jax.lax.dot_general(qh, kbuf[slot], (((1,), (1,)), ((), ())),
                                        preferred_element_type=f32) * scale
                m_new = jnp.maximum(m, jnp.max(s, axis=-1, keepdims=True))
                alpha = jnp.exp(m - m_new)
                p = jnp.exp(s - m_new)
                l = alpha * l + jnp.sum(p, axis=-1, keepdims=True)
                vcopy(0, slot).wait()
                pv = jnp.dot(p.astype(bf16), vbuf[slot], preferred_element_type=f32)
                acc = alpha * acc + pv
                nxt = step + nbuf

                @pl.when(nxt < total)
                def _():
                    nh = nxt // (B * ns)
                    rem = nxt - nh * (B * ns)
                    nb = rem // ns
                    ni = rem - nb * ns
                    src = (nb * H + nh) * ns + ni
                    kcopy(src, slot).start()
                    vcopy(src, slot).start()

                return m_new, l, acc

            m0 = jnp.full((MP, 1), -jnp.inf, f32)
            l0 = jnp.zeros((MP, 1), f32)
            a0 = jnp.zeros((MP, DH), f32)
            m, l, acc = jax.lax.fori_loop(0, ns, chunk, (m0, l0, a0))
            o_s[hh] = jnp.where(row == b, acc / l, o_s[hh])
            return 0

        jax.lax.fori_loop(0, B, batch_loop, 0)
        return 0

    jax.lax.fori_loop(0, H, head_loop, 0)

    wo_c.wait()
    wg_c.wait()
    wu_c.wait()
    wd_c.wait()
    o = jnp.concatenate([o_s[hh] for hh in range(H)], axis=-1).astype(bf16)
    wr_c.wait()
    nt = (((1,), (1,)), ((), ()))
    attn = jax.lax.dot_general(o, wo_v[...], nt, preferred_element_type=f32)
    x = x + ga * attn
    h = _layernorm(x) * (1.0 + cb) + sb
    hb = h.astype(bf16)
    r = jnp.sum(hb.astype(f32) * wr_ref[...].astype(f32).reshape(1, D), axis=-1, keepdims=True)
    g = _silu(jnp.dot(hb, wg_v[...], preferred_element_type=f32))
    u = jnp.dot(hb, wu_v[...], preferred_element_type=f32)
    y = jax.lax.dot_general((g * u).astype(bf16), wd_v[...], nt, preferred_element_type=f32)
    y = y * (1.0 / (1.0 + jnp.exp(-r)))
    res = x + gb * (h + (h * 0.0 + y))
    out_ref[...] = res[:B].astype(out_ref.dtype)
    out_c = pltpu.make_async_copy(out_ref, out_hbm, wsem.at[9])
    out_c.start()
    out_c.wait()


def _make(bs, nbuf):
    def run(A_x, A_k_cache, A_v_cache, A_wq, A_wo, B_x, B_w_r, B_w_gate, B_w_up, B_w_down, c, w_mod):
        del B_x
        k2 = A_k_cache.reshape(B * H * SK, DH)
        v2 = A_v_cache.reshape(B * H * SK, DH)
        bf16 = jnp.bfloat16
        hbm = pl.BlockSpec(memory_space=pltpu.HBM)
        return pl.pallas_call(
            functools.partial(_kernel, bs=bs, nbuf=nbuf),
            out_shape=jax.ShapeDtypeStruct((B, D), A_x.dtype),
            in_specs=[hbm] * 11,
            out_specs=hbm,
            scratch_shapes=[
                pltpu.VMEM((B, D), bf16),
                pltpu.VMEM((B, D), bf16),
                pltpu.VMEM((D,), bf16),
                pltpu.VMEM((B, D), A_x.dtype),
                pltpu.VMEM((nbuf, bs, DH), bf16),
                pltpu.VMEM((nbuf, bs, DH), bf16),
                pltpu.VMEM((D, H * DH), bf16),
                pltpu.VMEM((D, H * DH), bf16),
                pltpu.VMEM((D, F), bf16),
                pltpu.VMEM((D, F), bf16),
                pltpu.VMEM((D, F), bf16),
                pltpu.VMEM((D, 6 * D), bf16),
                pltpu.VMEM((H, MP, DH), bf16),
                pltpu.VMEM((H, MP, DH), jnp.float32),
                pltpu.SemaphoreType.DMA((nbuf,)),
                pltpu.SemaphoreType.DMA((nbuf,)),
                pltpu.SemaphoreType.DMA((10,)),
            ],
            compiler_params=pltpu.CompilerParams(vmem_limit_bytes=100 * 1024 * 1024),
        )(A_x.reshape(B, D), c, B_w_r, k2, v2, A_wq, A_wo.T, B_w_gate, B_w_up, B_w_down.T,
          w_mod).reshape(B, 1, D)
    return run


@jax.jit
def pallas_adaLN_cond__mha_block_cached__moe_arch_mod__decode_kernel(
    A_x: jax.Array,
    A_k_cache: jax.Array,
    A_v_cache: jax.Array,
    A_wq: jax.Array,
    A_wo: jax.Array,
    B_x: jax.Array,
    B_w_r: jax.Array,
    B_w_gate: jax.Array,
    B_w_up: jax.Array,
    B_w_down: jax.Array,
    c: jax.Array,
    w_mod: jax.Array,
):
    return _make(2048, 4)(A_x, A_k_cache, A_v_cache, A_wq, A_wo, B_x, B_w_r,
                          B_w_gate, B_w_up, B_w_down, c, w_mod)
```

```python
import functools

import jax
import jax.numpy as jnp
import jax.experimental.pallas as pl
import jax.experimental.pallas.tpu as pltpu

B, D, H, SK, DH, F = 4, 448, 16, 16384, 256, 1792
MP = 8


def _silu(v):
    return v * (1.0 / (1.0 + jnp.exp(-v)))


def _layernorm(v):
    m = jnp.mean(v, axis=-1, keepdims=True)
    d = v - m
    var = jnp.mean(d * d, axis=-1, keepdims=True)
    return d / jnp.sqrt(var + 1e-5)


def _pad_rows(v):
    return jnp.concatenate([v, jnp.zeros((MP - v.shape[0], v.shape[1]), v.dtype)], axis=0)


def _kernel(x_hbm, c_hbm, wr_hbm,
            k_hbm, v_hbm, wq_hbm, wo_hbm, wg_hbm, wu_hbm, wd_hbm, wm_hbm,
            out_hbm,
            x_ref, c_ref, wr_ref, out_ref,
            kbuf, vbuf, wq_v, wo_v, wg_v, wu_v, wd_v, wm_v, q_s, o_s,
            ksem, vsem, wsem, *, bs, sub, nbuf):
    ns = SK // bs
    total = B * H * ns
    f32 = jnp.float32
    bf16 = jnp.bfloat16

    def kv_start(j, slot):
        for t in range(bs // sub):
            src = pl.ds(j * bs + t * sub, sub)
            dst = pl.ds(t * sub, sub)
            pltpu.make_async_copy(k_hbm.at[src, :], kbuf.at[slot, dst, :], ksem.at[slot]).start(priority=0)
            pltpu.make_async_copy(v_hbm.at[src, :], vbuf.at[slot, dst, :], vsem.at[slot]).start(priority=1)

    def k_wait(slot):
        pltpu.make_async_copy(kbuf.at[slot], kbuf.at[slot], ksem.at[slot]).wait()

    def v_wait(slot):
        pltpu.make_async_copy(vbuf.at[slot], vbuf.at[slot], vsem.at[slot]).wait()

    def w_start(src, dst, sem):
        for t in range(D // 16):
            rows = pl.ds(t * 16, 16)
            pltpu.make_async_copy(src.at[rows, :], dst.at[rows, :], sem).start(priority=t % 2)

    def w_wait(dst, sem):
        pltpu.make_async_copy(dst, dst, sem).wait()

    x_c = pltpu.make_async_copy(x_hbm, x_ref, wsem.at[6])
    c_c = pltpu.make_async_copy(c_hbm, c_ref, wsem.at[7])
    wr_c = pltpu.make_async_copy(wr_hbm, wr_ref, wsem.at[8])
    x_c.start()
    c_c.start(priority=1)
    wr_c.start()
    w_start(wm_hbm, wm_v, wsem.at[0])
    w_start(wq_hbm, wq_v, wsem.at[1])
    for j in range(nbuf):
        kv_start(j, j)
    w_start(wo_hbm, wo_v, wsem.at[2])
    w_start(wg_hbm, wg_v, wsem.at[3])
    w_start(wu_hbm, wu_v, wsem.at[4])
    w_start(wd_hbm, wd_v, wsem.at[5])

    x_c.wait()
    c_c.wait()
    x = _pad_rows(x_ref[...].astype(f32))
    c = _pad_rows(c_ref[...].astype(f32))
    sc = _silu(c).astype(bf16)
    w_wait(wm_v, wsem.at[0])
    mod = jnp.dot(sc, wm_v[...], preferred_element_type=f32)
    sa, ca, ga, sb, cb, gb = [mod[:, i * D:(i + 1) * D] for i in range(6)]
    h = _layernorm(x) * (1.0 + ca) + sa
    w_wait(wq_v, wsem.at[1])
    q = jnp.dot(h.astype(bf16), wq_v[...], preferred_element_type=f32)
    q = q.astype(bf16)
    for hh in range(H):
        q_s[hh] = q[:, hh * DH:(hh + 1) * DH]

    scale = DH ** -0.5
    row = jax.lax.broadcasted_iota(jnp.int32, (MP, DH), 0)

    for hh in range(H):
        o_s[hh] = jnp.zeros((MP, DH), f32)

    def head_loop(bh, _):
        b = bh // H
        hh = bh - b * H
        qh = q_s[hh]

        def chunk(i, carry):
            m, l, acc = carry
            step = bh * ns + i
            slot = jax.lax.rem(step, nbuf)
            k_wait(slot)
            s = jax.lax.dot_general(qh, kbuf[slot], (((1,), (1,)), ((), ())),
                                    preferred_element_type=f32) * scale
            m_new = jnp.maximum(m, jnp.max(s, axis=-1, keepdims=True))
            alpha = jnp.exp(m - m_new)
            p = jnp.exp(s - m_new)
            l = alpha * l + jnp.sum(p, axis=-1, keepdims=True)
            v_wait(slot)
            pv = jnp.dot(p.astype(bf16), vbuf[slot], preferred_element_type=f32)
            acc = alpha * acc + pv

            @pl.when(step + nbuf < total)
            def _():
                kv_start(step + nbuf, slot)

            return m_new, l, acc

        m0 = jnp.full((MP, 1), -jnp.inf, f32)
        l0 = jnp.zeros((MP, 1), f32)
        a0 = jnp.zeros((MP, DH), f32)
        m, l, acc = jax.lax.fori_loop(0, ns, chunk, (m0, l0, a0))
        o_s[hh] = jnp.where(row == b, acc / l, o_s[hh])
        return 0

    jax.lax.fori_loop(0, B * H, head_loop, 0)

    w_wait(wo_v, wsem.at[2])
    w_wait(wg_v, wsem.at[3])
    w_wait(wu_v, wsem.at[4])
    w_wait(wd_v, wsem.at[5])
    o = jnp.concatenate([o_s[hh] for hh in range(H)], axis=-1).astype(bf16)
    wr_c.wait()
    nt = (((1,), (1,)), ((), ()))
    attn = jax.lax.dot_general(o, wo_v[...], nt, preferred_element_type=f32)
    x = x + ga * attn
    h = _layernorm(x) * (1.0 + cb) + sb
    hb = h.astype(bf16)
    r = jnp.sum(hb.astype(f32) * wr_ref[...].astype(f32).reshape(1, D), axis=-1, keepdims=True)
    g = _silu(jnp.dot(hb, wg_v[...], preferred_element_type=f32))
    u = jnp.dot(hb, wu_v[...], preferred_element_type=f32)
    y = jax.lax.dot_general((g * u).astype(bf16), wd_v[...], nt, preferred_element_type=f32)
    y = y * (1.0 / (1.0 + jnp.exp(-r)))
    res = x + gb * (h + (h * 0.0 + y))
    out_ref[...] = res[:B].astype(out_ref.dtype)
    out_c = pltpu.make_async_copy(out_ref, out_hbm, wsem.at[9])
    out_c.start()
    out_c.wait()


def _make(bs, sub, nbuf):
    def run(A_x, A_k_cache, A_v_cache, A_wq, A_wo, B_x, B_w_r, B_w_gate, B_w_up, B_w_down, c, w_mod):
        del B_x
        k2 = A_k_cache.reshape(B * H * SK, DH)
        v2 = A_v_cache.reshape(B * H * SK, DH)
        bf16 = jnp.bfloat16
        hbm = pl.BlockSpec(memory_space=pltpu.HBM)
        return pl.pallas_call(
            functools.partial(_kernel, bs=bs, sub=sub, nbuf=nbuf),
            out_shape=jax.ShapeDtypeStruct((B, D), A_x.dtype),
            in_specs=[hbm] * 11,
            out_specs=hbm,
            scratch_shapes=[
                pltpu.VMEM((B, D), bf16),
                pltpu.VMEM((B, D), bf16),
                pltpu.VMEM((D,), bf16),
                pltpu.VMEM((B, D), A_x.dtype),
                pltpu.VMEM((nbuf, bs, DH), bf16),
                pltpu.VMEM((nbuf, bs, DH), bf16),
                pltpu.VMEM((D, H * DH), bf16),
                pltpu.VMEM((D, H * DH), bf16),
                pltpu.VMEM((D, F), bf16),
                pltpu.VMEM((D, F), bf16),
                pltpu.VMEM((D, F), bf16),
                pltpu.VMEM((D, 6 * D), bf16),
                pltpu.VMEM((H, MP, DH), bf16),
                pltpu.VMEM((H, MP, DH), jnp.float32),
                pltpu.SemaphoreType.DMA((nbuf,)),
                pltpu.SemaphoreType.DMA((nbuf,)),
                pltpu.SemaphoreType.DMA((10,)),
            ],
            compiler_params=pltpu.CompilerParams(vmem_limit_bytes=100 * 1024 * 1024),
        )(A_x.reshape(B, D), c, B_w_r, k2, v2, A_wq, A_wo.T, B_w_gate, B_w_up, B_w_down.T,
          w_mod).reshape(B, 1, D)
    return run


@jax.jit
def pallas_adaLN_cond__mha_block_cached__moe_arch_mod__decode_kernel(
    A_x: jax.Array,
    A_k_cache: jax.Array,
    A_v_cache: jax.Array,
    A_wq: jax.Array,
    A_wo: jax.Array,
    B_x: jax.Array,
    B_w_r: jax.Array,
    B_w_gate: jax.Array,
    B_w_up: jax.Array,
    B_w_down: jax.Array,
    c: jax.Array,
    w_mod: jax.Array,
):
    return _make(1024, 64, 4)(A_x, A_k_cache, A_v_cache, A_wq, A_wo, B_x, B_w_r,
                          B_w_gate, B_w_up, B_w_down, c, w_mod)
```

```python
import functools

import jax
import jax.numpy as jnp
import jax.experimental.pallas as pl
import jax.experimental.pallas.tpu as pltpu

B, D, H, SK, DH, F = 4, 448, 16, 16384, 256, 1792
MP = 8


def _silu(v):
    return v * (1.0 / (1.0 + jnp.exp(-v)))


def _layernorm(v):
    m = jnp.mean(v, axis=-1, keepdims=True)
    d = v - m
    var = jnp.mean(d * d, axis=-1, keepdims=True)
    return d / jnp.sqrt(var + 1e-5)


def _pad_rows(v):
    return jnp.concatenate([v, jnp.zeros((MP - v.shape[0], v.shape[1]), v.dtype)], axis=0)


def _kernel(x_hbm, c_hbm, wr_hbm,
            k_hbm, v_hbm, wq_hbm, wo_hbm, wg_hbm, wu_hbm, wd_hbm, wm_hbm,
            out_hbm,
            x_ref, c_ref, wr_ref, out_ref,
            kbuf, vbuf, wq_v, wo_v, wg_v, wu_v, wd_v, wm_v, q_s, o_s,
            ksem, vsem, wsem, *, bs, sub, nbuf):
    ns = SK // bs
    total = B * H * ns
    f32 = jnp.float32
    bf16 = jnp.bfloat16

    def kv_start(j, slot):
        for t in range(0, bs, sub):
            n = min(sub, bs - t)
            src = pl.ds(j * bs + t, n)
            dst = pl.ds(t, n)
            pltpu.make_async_copy(k_hbm.at[src, :], kbuf.at[slot, dst, :], ksem.at[slot]).start(priority=0)
            pltpu.make_async_copy(v_hbm.at[src, :], vbuf.at[slot, dst, :], vsem.at[slot]).start(priority=1)

    def k_wait(slot):
        pltpu.make_async_copy(kbuf.at[slot], kbuf.at[slot], ksem.at[slot]).wait()

    def v_wait(slot):
        pltpu.make_async_copy(vbuf.at[slot], vbuf.at[slot], vsem.at[slot]).wait()

    def w_start(src, dst, sem):
        width = dst.shape[1]
        cuts = {H * DH: (0, 1408, 2816, width), 6 * D: (0, 1408, width)}.get(width, (0, width))
        for t in range(D // 16):
            rows = pl.ds(t * 16, 16)
            for lo, hi in zip(cuts[:-1], cuts[1:]):
                cols = pl.ds(lo, hi - lo)
                pltpu.make_async_copy(src.at[rows, cols], dst.at[rows, cols], sem).start(priority=t % 2)

    def w_wait(dst, sem):
        pltpu.make_async_copy(dst, dst, sem).wait()

    x_c = pltpu.make_async_copy(x_hbm, x_ref, wsem.at[6])
    c_c = pltpu.make_async_copy(c_hbm, c_ref, wsem.at[7])
    wr_c = pltpu.make_async_copy(wr_hbm, wr_ref, wsem.at[8])
    x_c.start()
    c_c.start(priority=1)
    wr_c.start()
    w_start(wm_hbm, wm_v, wsem.at[0])
    w_start(wq_hbm, wq_v, wsem.at[1])
    for j in range(nbuf):
        kv_start(j, j)

    x_c.wait()
    c_c.wait()
    x = _pad_rows(x_ref[...].astype(f32))
    c = _pad_rows(c_ref[...].astype(f32))
    sc = _silu(c).astype(bf16)
    w_wait(wm_v, wsem.at[0])
    mod = jnp.dot(sc, wm_v[...], preferred_element_type=f32)
    sa, ca, ga, sb, cb, gb = [mod[:, i * D:(i + 1) * D] for i in range(6)]
    h = _layernorm(x) * (1.0 + ca) + sa
    w_wait(wq_v, wsem.at[1])
    q = jnp.dot(h.astype(bf16), wq_v[...], preferred_element_type=f32)
    q = q.astype(bf16)
    for hh in range(H):
        q_s[hh] = q[:, hh * DH:(hh + 1) * DH]

    scale = DH ** -0.5
    row = jax.lax.broadcasted_iota(jnp.int32, (MP, DH), 0)

    for hh in range(H):
        o_s[hh] = jnp.zeros((MP, DH), f32)

    def head_loop(bh, _):
        b = bh // H
        hh = bh - b * H
        qh = q_s[hh]

        def chunk(i, carry):
            m, l, acc = carry
            step = bh * ns + i
            slot = jax.lax.rem(step, nbuf)
            k_wait(slot)
            s = jax.lax.dot_general(qh, kbuf[slot], (((1,), (1,)), ((), ())),
                                    preferred_element_type=f32) * scale
            m_new = jnp.maximum(m, jnp.max(s, axis=-1, keepdims=True))
            alpha = jnp.exp(m - m_new)
            p = jnp.exp(s - m_new)
            l = alpha * l + jnp.sum(p, axis=-1, keepdims=True)
            v_wait(slot)
            pv = jnp.dot(p.astype(bf16), vbuf[slot], preferred_element_type=f32)
            acc = alpha * acc + pv

            @pl.when(step + nbuf < total)
            def _():
                kv_start(step + nbuf, slot)

            @pl.when(step + nbuf == total)
            def _():
                w_start(wo_hbm, wo_v, wsem.at[2])
                w_start(wg_hbm, wg_v, wsem.at[3])
                w_start(wu_hbm, wu_v, wsem.at[4])
                w_start(wd_hbm, wd_v, wsem.at[5])

            return m_new, l, acc

        m0 = jnp.full((MP, 1), -jnp.inf, f32)
        l0 = jnp.zeros((MP, 1), f32)
        a0 = jnp.zeros((MP, DH), f32)
        m, l, acc = jax.lax.fori_loop(0, ns, chunk, (m0, l0, a0))
        o_s[hh] = jnp.where(row == b, acc / l, o_s[hh])
        return 0

    jax.lax.fori_loop(0, B * H, head_loop, 0)

    w_wait(wo_v, wsem.at[2])
    o = jnp.concatenate([o_s[hh] for hh in range(H)], axis=-1).astype(bf16)
    wr_c.wait()
    nt = (((1,), (1,)), ((), ()))
    attn = jax.lax.dot_general(o, wo_v[...], nt, preferred_element_type=f32)
    x = x + ga * attn
    h = _layernorm(x) * (1.0 + cb) + sb
    hb = h.astype(bf16)
    r = jnp.sum(hb.astype(f32) * wr_ref[...].astype(f32).reshape(1, D), axis=-1, keepdims=True)
    w_wait(wg_v, wsem.at[3])
    g = _silu(jnp.dot(hb, wg_v[...], preferred_element_type=f32))
    w_wait(wu_v, wsem.at[4])
    u = jnp.dot(hb, wu_v[...], preferred_element_type=f32)
    w_wait(wd_v, wsem.at[5])
    y = jax.lax.dot_general((g * u).astype(bf16), wd_v[...], nt, preferred_element_type=f32)
    y = y * (1.0 / (1.0 + jnp.exp(-r)))
    res = x + gb * (h + (h * 0.0 + y))
    out_ref[...] = res[:B].astype(out_ref.dtype)
    out_c = pltpu.make_async_copy(out_ref, out_hbm, wsem.at[9])
    out_c.start()
    out_c.wait()


def _make(bs, sub, nbuf):
    def run(A_x, A_k_cache, A_v_cache, A_wq, A_wo, B_x, B_w_r, B_w_gate, B_w_up, B_w_down, c, w_mod):
        del B_x
        k2 = A_k_cache.reshape(B * H * SK, DH)
        v2 = A_v_cache.reshape(B * H * SK, DH)
        bf16 = jnp.bfloat16
        hbm = pl.BlockSpec(memory_space=pltpu.HBM)
        return pl.pallas_call(
            functools.partial(_kernel, bs=bs, sub=sub, nbuf=nbuf),
            out_shape=jax.ShapeDtypeStruct((B, D), A_x.dtype),
            in_specs=[hbm] * 11,
            out_specs=hbm,
            scratch_shapes=[
                pltpu.VMEM((B, D), bf16),
                pltpu.VMEM((B, D), bf16),
                pltpu.VMEM((D,), bf16),
                pltpu.VMEM((B, D), A_x.dtype),
                pltpu.VMEM((nbuf, bs, DH), bf16),
                pltpu.VMEM((nbuf, bs, DH), bf16),
                pltpu.VMEM((D, H * DH), bf16),
                pltpu.VMEM((D, H * DH), bf16),
                pltpu.VMEM((D, F), bf16),
                pltpu.VMEM((D, F), bf16),
                pltpu.VMEM((D, F), bf16),
                pltpu.VMEM((D, 6 * D), bf16),
                pltpu.VMEM((H, MP, DH), bf16),
                pltpu.VMEM((H, MP, DH), jnp.float32),
                pltpu.SemaphoreType.DMA((nbuf,)),
                pltpu.SemaphoreType.DMA((nbuf,)),
                pltpu.SemaphoreType.DMA((10,)),
            ],
            compiler_params=pltpu.CompilerParams(vmem_limit_bytes=100 * 1024 * 1024),
        )(A_x.reshape(B, D), c, B_w_r, k2, v2, A_wq, A_wo.T, B_w_gate, B_w_up, B_w_down.T,
          w_mod).reshape(B, 1, D)
    return run


@jax.jit
def pallas_adaLN_cond__mha_block_cached__moe_arch_mod__decode_kernel(
    A_x: jax.Array,
    A_k_cache: jax.Array,
    A_v_cache: jax.Array,
    A_wq: jax.Array,
    A_wo: jax.Array,
    B_x: jax.Array,
    B_w_r: jax.Array,
    B_w_gate: jax.Array,
    B_w_up: jax.Array,
    B_w_down: jax.Array,
    c: jax.Array,
    w_mod: jax.Array,
):
    return _make(1024, 96, 6)(A_x, A_k_cache, A_v_cache, A_wq, A_wo, B_x, B_w_r,
                          B_w_gate, B_w_up, B_w_down, c, w_mod)
```
